```python
import os as _os
_os.environ.setdefault("JAX_PLATFORMS", "cpu")
import jax
import jax.numpy as jnp

def _softmax(x, axis=-1):
    return jax.nn.softmax(x, axis=axis)
def _gelu(x):
    return jax.nn.gelu(x, approximate=True)
def _silu(x):
    return jax.nn.silu(x)
def _sigmoid(x):
    return jax.nn.sigmoid(x)
def _layernorm(x, axis=-1, eps=1e-5):
    m = jnp.mean(x, axis=axis, keepdims=True)
    v = jnp.var(x, axis=axis, keepdims=True)
    return (x - m) / jnp.sqrt(v + eps)
def _scatter_add(tgt, idx, src, axis=0):
    return tgt.at[idx].add(src)
def _segment_sum(src, seg, n):
    return jax.ops.segment_sum(src, seg, n)
class _Rng:
    def __init__(self, key):
        self._k = key
    def _next(self):
        self._k, sub = jax.random.split(self._k)
        return sub
    def normal(self, shape):
        return jax.random.normal(self._next(), shape, dtype=jnp.bfloat16)
    def randint(self, lo, hi, shape):
        return jax.random.randint(self._next(), shape, lo, hi, dtype=jnp.int32)
    def uniform(self, shape, lo=0.0, hi=1.0):
        return jax.random.uniform(self._next(), shape, jnp.bfloat16, lo, hi)
    def permutation(self, n):
        return jax.random.permutation(self._next(), n)


kernel_name = 'parallel_sum__softmax_full_mha__moe_arch_mod__prompt'

def setup_inputs():
    _rng = _Rng(jax.random.key(int.from_bytes(__import__("os").urandom(4), "little")))
    _w = (lambda a: (lambda t: t.astype(jnp.bfloat16) if jnp.issubdtype(t.dtype, jnp.floating) else t)(jnp.asarray(a)))
    def _A_setup():
        B, S, D = 1, 2048, 512
        return {
            "x": _w((lambda *s: _rng.normal(s) * 0.05)(B, S, D)),
            "wqkv": _w((lambda *s: _rng.normal(s) * 0.1)(D, 3 * D)),
            "wo": _w((lambda *s: _rng.normal(s) * 0.05)(D, D)),
        }
    _A_in = _A_setup()

    def _B_setup():
        B, S, D, F, C = 1, 2048, 512, 1792, 1
        return {
            "x": _w((lambda *s: _rng.normal(s) * 0.05)(B, S, D)),
            "w_r": _w((lambda *s: _rng.normal(s) * 1.6)(D)),
            "w_gate": _w((lambda *s: _rng.normal(s) * 0.1)(D, F)),
            "w_up": _w((lambda *s: _rng.normal(s) * 0.1)(D, F)),
            "w_down": _w((lambda *s: _rng.normal(s) * 0.1)(F, D)),
        }
    _B_in = _B_setup()

    return {
        "A_x": _A_in["x"],
        "A_wqkv": _A_in["wqkv"],
        "A_wo": _A_in["wo"],
        "B_x": _B_in["x"],
        "B_w_r": _B_in["w_r"],
        "B_w_gate": _B_in["w_gate"],
        "B_w_up": _B_in["w_up"],
        "B_w_down": _B_in["w_down"],
    }

def reference(A_x, A_wqkv, A_wo, B_x, B_w_r, B_w_gate, B_w_up, B_w_down):
    def _A_ref(x, wqkv, wo):
        B, S, D = x.shape
        H = 32; Dh = D // H
        qkv = (lambda x, *d: x.transpose(*d))((x @ wqkv).reshape(B, S, 3, H, Dh), 2, 0, 3, 1, 4)
        q, k, v = qkv[0], qkv[1], qkv[2]
        scale = Dh ** -0.5
        scores = jnp.einsum("bhqd,bhkd->bhqk", q, k) * scale
        p = _softmax(scores, axis=-1)
        o = jnp.einsum("bhqk,bhkd->bhqd", p, v)
        return (lambda x, *d: x.transpose(*d))(o, 0, 2, 1, 3).reshape(B, S, D) @ wo

    def _B_ref(x, w_r, w_gate, w_up, w_down):
        B, S, D = x.shape
        C = 1
        r = x @ w_r
        idx = jnp.argsort(-r, axis=-1)[:, :C]
        idx_e = jnp.repeat(idx.reshape(B, C, 1), D, axis=2)
        x_sel = jnp.take_along_axis(x, idx_e, axis=1)
        g = _silu(x_sel @ w_gate)
        u = x_sel @ w_up
        y = (g * u) @ w_down
        r_sel = _sigmoid(jnp.take_along_axis(r, idx, axis=1))
        y = y * r_sel.reshape(B, C, 1)
        b_off = (jnp.arange(B) * S).reshape(B, 1)
        flat_idx = (idx + b_off).reshape(B * C)
        zero = (x * 0.0).reshape(B * S, D)
        upd = _scatter_add(zero, flat_idx, y.reshape(B * C, D), axis=0)
        return x + upd.reshape(B, S, D)

    x = A_x
    xn = _layernorm(x, axis=-1)
    return x + _A_ref(xn, A_wqkv, A_wo) + _B_ref(xn, B_w_r, B_w_gate, B_w_up, B_w_down)
```

```python
import functools
import math

import jax
import jax.numpy as jnp
from jax import lax
import jax.experimental.pallas as pl
import jax.experimental.pallas.tpu as pltpu

H = 32
LANES = 128
F32 = jnp.float32
BF16 = jnp.bfloat16

CFG = dict(TQ=512, KC=128, RC=512, LAG=1, TK=1, OC=512)


def _dot(a, b):
    return jnp.dot(a, b, preferred_element_type=F32)


def _dot_nt(a, b):
    return lax.dot_general(a, b, (((1,), (1,)), ((), ())), preferred_element_type=F32)


def _dot_tn(a, b):
    return lax.dot_general(a, b, (((0,), (0,)), ((), ())), preferred_element_type=F32)


def _kernel(x_hbm, wqkv_hbm, wo_hbm, wr_hbm, wg_hbm, wu_hbm, wd_hbm, out_hbm,
            x_s, wqkv_s, wo_s, wr_s, wg_s, wu_s, wd_s, out_s,
            xn_s, res_s, wt_s, qt_s, k_s, vt_s, r_s, sa_s, sb_s, ot_s, flag_s,
            sems, osems, *, S, D, cfg):
    TQ, KC, RC, LAG, TK, OC = (cfg[k] for k in ("TQ", "KC", "RC", "LAG", "TK", "OC"))
    DH = D // H
    HG = LANES // DH
    NG = D // LANES
    NRC = S // RC
    NC = S // KC
    NQ = S // TQ
    qscale = (DH ** -0.5) * math.log2(math.e)

    def cp(src, dst, i):
        return pltpu.make_async_copy(src, dst, sems.at[i])
    x_cp = [cp(x_hbm.at[pl.ds(c * RC, RC)], x_s.at[pl.ds(c * RC, RC)], c) for c in range(NRC)]
    w_cp = cp(wqkv_hbm, wqkv_s, NRC)
    wr_cp = cp(wr_hbm, wr_s, NRC + 1)
    wg_cp = cp(wg_hbm, wg_s, NRC + 2)
    wu_cp = cp(wu_hbm, wu_s, NRC + 3)
    wd_cp = cp(wd_hbm, wd_s, NRC + 4)
    wo_cp = cp(wo_hbm, wo_s, NRC + 5)
    x_cp[0].start()
    w_cp.start()
    wr_cp.start()
    for c in range(1, NRC):
        x_cp[c].start()
    wg_cp.start()
    wu_cp.start()
    wd_cp.start()
    wo_cp.start()
    flag_s[0] = 0

    def ln(c):
        rows = pl.ds(c * RC, RC)
        xb = x_s[rows, :]
        xf = xb.astype(F32)
        mean = jnp.mean(xf, axis=-1, keepdims=True)
        cen = xf - mean
        var = jnp.mean(cen * cen, axis=-1, keepdims=True)
        xn = (cen * lax.rsqrt(var + 1e-5)).astype(BF16)
        xn_s[rows, :] = xn
        res_s[rows, :] = xf + xn.astype(F32)
        return xn

    x_cp[0].wait()
    xn = ln(0)
    w_cp.wait()
    wr_cp.wait()
    wt_s[0:D, :] = wqkv_s[:, 0:D].T
    wt_s[D:2 * D, :] = wqkv_s[:, 2 * D:3 * D].T
    wt_s[2 * D:2 * D + 16, :] = jnp.broadcast_to(wr_s[...], (16, D))
    for c in range(NRC):
        cols = pl.ds(c * RC, RC)
        kk = _dot(xn, wqkv_s[:, D:2 * D]).astype(BF16)
        for g in range(NG):
            k_s[g, cols, :] = kk[:, g * LANES:(g + 1) * LANES]
        t = _dot_nt(wt_s[...], xn)
        qt_s[:, cols] = (t[0:D] * qscale).astype(BF16)
        vt_s[:, cols] = t[D:2 * D].astype(BF16)
        r_s[:, cols] = t[2 * D:2 * D + 8]
        if c + 1 < NRC:
            x_cp[c + 1].wait()
            xn = ln(c + 1)

    r = r_s[0:1, :].astype(BF16).astype(F32)
    rmax = jnp.max(r, axis=-1, keepdims=True)
    tok = lax.broadcasted_iota(jnp.int32, (1, S), 1)
    idx = jnp.min(jnp.where(r == rmax, tok, S - 1))
    blk = pl.multiple_of((idx // 16) * 16, 16)
    xsel = xn_s[pl.ds(blk, 16), :]
    wg_cp.wait()
    wu_cp.wait()
    gate = _dot(xsel, wg_s[...]).astype(BF16).astype(F32)
    up = _dot(xsel, wu_s[...]).astype(BF16).astype(F32)
    hid = (gate * jax.nn.sigmoid(gate)).astype(BF16).astype(F32) * up
    wd_cp.wait()
    y = _dot(hid.astype(BF16), wd_s[...]) * jax.nn.sigmoid(rmax)
    row = lax.broadcasted_iota(jnp.int32, (16, D), 0) + blk
    res_s[pl.ds(blk, 16), :] = res_s[pl.ds(blk, 16), :] + jnp.where(row == idx, y, 0.0)

    def q_weights(h, t0, sub):
        q = qt_s[pl.ds(pl.multiple_of(h * DH, DH), DH), pl.ds(t0, TQ)]
        parts = []
        if sub > 0:
            parts.append(jnp.zeros((DH * sub, TQ), BF16))
        parts.append(q)
        if sub < HG - 1:
            parts.append(jnp.zeros((DH * (HG - 1 - sub), TQ), BF16))
        return jnp.concatenate(parts, axis=0)

    def qk_chunk(g, qm, c, dst):
        s = _dot(k_s[g, c * KC:(c + 1) * KC, :], qm)
        dst[c * KC:(c + 1) * KC, :] = s
        return jnp.max(s.reshape(KC // 8, 8, TQ), axis=0), s[KC - 8:, :]

    def pv_chunk(h, m8, c, src):
        s = src[c * KC:(c + 1) * KC, :]
        m = jnp.broadcast_to(m8[None], (KC // 8, 8, TQ)).reshape(KC, TQ)
        p = jnp.exp2(s - m)
        l = None
        for kt in range(KC // LANES):
            for rr in reversed(range(LANES // 16)):
                b = kt * LANES + rr * 16
                t = p[b + 8:b + 16] + p[b:b + 8]
                l = t if l is None else l + t
        o = _dot(vt_s[pl.ds(pl.multiple_of(h * DH, DH), DH), c * KC:(c + 1) * KC], p.astype(BF16))
        return l, o

    def step(j, sub, mprev, src, dst):
        t0 = pl.multiple_of((j // NG) * TQ, TQ)
        h = (j % NG) * HG + sub
        if sub < HG - 1:
            gn, hn, tn = j % NG, h + 1, t0
        else:
            jn = jnp.minimum(j + 1, NQ * NG - 1)
            gn = jn % NG
            hn, tn = gn * HG, pl.multiple_of((jn // NG) * TQ, TQ)
        qm = q_weights(hn, tn, (sub + 1) % HG)
        mb = jnp.broadcast_to(jnp.max(mprev, axis=0, keepdims=True), (8, TQ))
        never = flag_s[0] > 0
        m = l = o = None
        lasts = []
        for c in range(NC + LAG):
            if c < NC:
                mc, last = qk_chunk(gn, qm, c, dst)
                lasts.append(last)
                m = mc if m is None else jnp.maximum(m, mc)
            if c >= LAG:
                cc = c - LAG
                mu = mb
                if TK >= 0 and 0 <= cc - TK < len(lasts):
                    mu = jnp.where(never, lasts[cc - TK], mu)
                lc, oc = pv_chunk(h, mu, cc, src)
                l = lc if l is None else l + lc
                o = oc if o is None else o + oc
        l = jnp.sum(l, axis=0, keepdims=True)
        ot_s[pl.ds(pl.multiple_of(h * DH, DH), DH), pl.ds(t0, TQ)] = (o / l).astype(BF16)
        return m

    qm0 = q_weights(0, 0, 0)
    m0 = None
    for c in range(NC):
        mc, _ = qk_chunk(0, qm0, c, sa_s)
        m0 = mc if m0 is None else jnp.maximum(m0, mc)

    def body(j, m):
        for sub in range(HG):
            a, b = (sa_s, sb_s) if sub % 2 == 0 else (sb_s, sa_s)
            m = step(j, sub, m, a, b)
        return m

    lax.fori_loop(0, NQ * NG, body, m0)

    wo_cp.wait()
    o_cp = []
    for c in range(S // OC):
        rows = pl.ds(c * OC, OC)
        a = _dot_tn(ot_s[:, rows], wo_s[...])
        out_s[rows, :] = (a + res_s[rows, :]).astype(BF16)
        o_cp.append(pltpu.make_async_copy(out_s.at[rows], out_hbm.at[rows], osems.at[c]))
        o_cp[-1].start()
    for d in o_cp:
        d.wait()


def make(cfg=None):
    cfg = dict(CFG, **(cfg or {}))

    def fn(A_x, A_wqkv, A_wo, B_x, B_w_r, B_w_gate, B_w_up, B_w_down):
        del B_x
        B, S, D = A_x.shape
        F = B_w_gate.shape[1]
        TQ, RC = cfg["TQ"], cfg["RC"]
        anyspec = pl.BlockSpec(memory_space=pl.ANY)
        out = pl.pallas_call(
            functools.partial(_kernel, S=S, D=D, cfg=cfg),
            out_shape=jax.ShapeDtypeStruct((S, D), BF16),
            in_specs=[anyspec] * 7,
            out_specs=anyspec,
            scratch_shapes=[
                pltpu.VMEM((S, D), BF16), pltpu.VMEM((D, 3 * D), BF16), pltpu.VMEM((D, D), BF16),
                pltpu.VMEM((1, D), BF16), pltpu.VMEM((D, F), BF16), pltpu.VMEM((D, F), BF16),
                pltpu.VMEM((F, D), BF16), pltpu.VMEM((S, D), BF16),
                pltpu.VMEM((S, D), BF16), pltpu.VMEM((S, D), F32), pltpu.VMEM((2 * D + 16, D), BF16),
                pltpu.VMEM((D, S), BF16), pltpu.VMEM((D // LANES, S, LANES), BF16), pltpu.VMEM((D, S), BF16),
                pltpu.VMEM((8, S), F32), pltpu.VMEM((S, TQ), F32), pltpu.VMEM((S, TQ), F32),
                pltpu.VMEM((D, S), BF16), pltpu.SMEM((1,), jnp.int32),
                pltpu.SemaphoreType.DMA((S // RC + 6,)), pltpu.SemaphoreType.DMA((S // cfg["OC"],)),
            ],
            compiler_params=pltpu.CompilerParams(vmem_limit_bytes=100 * 1024 * 1024),
            name="fused_block",
        )(A_x.reshape(S, D), A_wqkv, A_wo, B_w_r.reshape(1, D), B_w_gate, B_w_up, B_w_down)
        return out.reshape(B, S, D)
    return fn


_impl = make()


@jax.jit
def pallas_parallel_sum__softmax_full_mha__moe_arch_mod__prompt_kernel(
    A_x: jax.Array,
    A_wqkv: jax.Array,
    A_wo: jax.Array,
    B_x: jax.Array,
    B_w_r: jax.Array,
    B_w_gate: jax.Array,
    B_w_up: jax.Array,
    B_w_down: jax.Array,
):
    return _impl(A_x, A_wqkv, A_wo, B_x, B_w_r, B_w_gate, B_w_up, B_w_down)
```

```python
import math

import jax
import jax.numpy as jnp
from jax import lax
import jax.experimental.pallas as pl
import jax.experimental.pallas.tpu as pltpu

H = 32
LANES = 128
F32 = jnp.float32
BF16 = jnp.bfloat16

TQ = 512
KC = 128
RC = 512
SPLIT = 384
OP = 128
OUT_DMAS = (6, 9, 12, 14, 15)


def _mo(v, n):
    return v if isinstance(v, int) else pl.multiple_of(v, n)


def _dot(a, b):
    return jnp.dot(a, b, preferred_element_type=F32)


def _dot_nt(a, b):
    return lax.dot_general(a, b, (((1,), (1,)), ((), ())), preferred_element_type=F32)


def _dot_tn(a, b):
    return lax.dot_general(a, b, (((0,), (0,)), ((), ())), preferred_element_type=F32)


def _kernel(x_hbm, wqkv_hbm, wo_hbm, wr_hbm, wg_hbm, wu_hbm, wd_hbm, out_hbm,
            x_s, wqkv_s, wo_s, wr_s, wg_s, wu_s, wd_s, out_s,
            xn_s, res_s, wt_s, qt_s, k_s, vt_s, r_s, sa_s, sb_s, ot_s, flag_s,
            sems, osems):
    S, D = x_s.shape
    FT = wg_s.shape[1]
    DH = D // H
    HG = LANES // DH
    NG = D // LANES
    NRC = S // RC
    NC = S // KC
    NJ = (S // TQ) * NG
    qscale = (DH ** -0.5) * math.log2(math.e)

    def cp(src, dst, i):
        return pltpu.make_async_copy(src, dst, sems.at[i])
    x_cp = [cp(x_hbm.at[pl.ds(c * RC, RC)], x_s.at[pl.ds(c * RC, RC)], c) for c in range(NRC)]
    w_cp = [cp(wqkv_hbm.at[:, pl.ds(i * D, D)], wqkv_s.at[:, pl.ds(i * D, D)], NRC + i)
            for i in range(3)]
    wr_cp = cp(wr_hbm, wr_s, NRC + 3)
    late_cp = [cp(wg_hbm, wg_s, NRC + 4), cp(wu_hbm, wu_s, NRC + 5),
               cp(wd_hbm, wd_s, NRC + 6), cp(wo_hbm, wo_s, NRC + 7)]
    for d in [x_cp[0], w_cp[1], w_cp[0], w_cp[2], wr_cp] + x_cp[1:]:
        d.start()
    flag_s[0] = 0
    sa_s[...] = jnp.zeros((S, TQ), F32)

    def ln(c):
        rows = pl.ds(c * RC, RC)
        xf = x_s[rows, :].astype(F32)
        cen = xf - jnp.mean(xf, axis=-1, keepdims=True)
        var = jnp.mean(cen * cen, axis=-1, keepdims=True)
        xn = (cen * lax.rsqrt(var + 1e-5)).astype(BF16)
        xn_s[rows, :] = xn
        res_s[rows, :] = xf + xn.astype(F32)
        return xn

    def proj_k(c, xn, lo=0, hi=RC):
        kk = _dot(xn[lo:hi], wqkv_s[:, D:2 * D]).astype(BF16)
        for g in range(NG):
            k_s[g, pl.ds(c * RC + lo, hi - lo), :] = kk[:, g * LANES:(g + 1) * LANES]

    x_cp[0].wait()
    xn = ln(0)
    w_cp[1].wait()
    proj_k(0, xn, 0, SPLIT)
    w_cp[0].wait()
    w_cp[2].wait()
    wr_cp.wait()
    for d in late_cp:
        d.start()
    wt_s[0:D, :] = wqkv_s[:, 0:D].T
    wt_s[D:2 * D, :] = wqkv_s[:, 2 * D:3 * D].T
    wt_s[2 * D:2 * D + 16, :] = jnp.broadcast_to(wr_s[...].reshape(1, D), (16, D))
    proj_k(0, xn, SPLIT, RC)
    waited = 1
    for c in range(NRC):
        cols = pl.ds(c * RC, RC)
        qt_s[:, cols] = (_dot_nt(wt_s[0:D, :], xn) * qscale).astype(BF16)
        while waited < min(NRC, max(c + 2, 3)):
            x_cp[waited].wait()
            waited += 1
        t = _dot_nt(wt_s[D:2 * D + 16, :], xn)
        vt_s[:, cols] = t[0:D].astype(BF16)
        r_s[:, cols] = t[D:D + 8]
        if c + 1 < NRC:
            xn = ln(c + 1)
            proj_k(c + 1, xn)

    def q_weights(h, t0, sub):
        q = qt_s[pl.ds(_mo(h * DH, DH), DH), pl.ds(t0, TQ)]
        parts = [jnp.zeros((DH * sub, TQ), BF16)] if sub > 0 else []
        parts.append(q)
        if sub < HG - 1:
            parts.append(jnp.zeros((DH * (HG - 1 - sub), TQ), BF16))
        return jnp.concatenate(parts, axis=0)

    class Step:
        def __init__(self, pv, qk, m_part, src, dst):
            self.pv, self.qk, self.src, self.dst = pv, qk, src, dst
            if qk is not None:
                self.qm = q_weights(*qk[1:])
            self.mb = jnp.broadcast_to(jnp.max(m_part, axis=0, keepdims=True), (8, TQ))
            self.never = flag_s[0] > 0
            self.m = self.l = self.o = None
            self.lasts = []

        def do_qk(self, c):
            s = _dot(k_s[self.qk[0], c * KC:(c + 1) * KC, :], self.qm)
            self.dst[c * KC:(c + 1) * KC, :] = s
            mc = jnp.max(s.reshape(KC // 8, 8, TQ), axis=0)
            self.m = mc if self.m is None else jnp.maximum(self.m, mc)
            self.lasts.append(s[KC - 8:, :])

        def do_pv(self, c):
            m8 = self.mb
            if 0 < c <= len(self.lasts):
                m8 = jnp.where(self.never, self.lasts[c - 1], m8)
            m = jnp.broadcast_to(m8[None], (KC // 8, 8, TQ)).reshape(KC, TQ)
            p = jnp.exp2(self.src[c * KC:(c + 1) * KC, :] - m)
            lc = None
            for b in reversed(range(0, KC, 8)):
                lc = p[b:b + 8] if lc is None else lc + p[b:b + 8]
            oc = _dot(vt_s[pl.ds(_mo(self.pv[0] * DH, DH), DH), c * KC:(c + 1) * KC],
                      p.astype(BF16))
            self.l = lc if self.l is None else self.l + lc
            self.o = oc if self.o is None else self.o + oc

        def finish(self):
            l = jnp.sum(self.l, axis=0, keepdims=True)
            ot_s[pl.ds(_mo(self.pv[1] * DH, DH), DH), pl.ds(self.pv[2], TQ)] = (
                self.o / l).astype(BF16)

    def item(j, sub):
        return j % NG, (j % NG) * HG + sub, _mo((j // NG) * TQ, TQ), sub

    def body(j, m):
        for sub in range(HG):
            a, b = (sa_s, sb_s) if sub % 2 == 0 else (sb_s, sa_s)
            if sub == 0:
                _, hp, tp, _ = item(jnp.maximum(j - 1, 0), HG - 1)
                pv = (hp, jnp.where(j > 0, hp, H), tp)
            else:
                _, hp, tp, _ = item(j, sub - 1)
                pv = (hp, hp, tp)
            st = Step(pv, item(j, sub), m, a, b)
            for c in range(NC + 1):
                if c < NC:
                    st.do_qk(c)
                if c >= 1:
                    st.do_pv(c - 1)
            st.finish()
            m = st.m
        return m

    m = lax.fori_loop(0, NJ, body, jnp.zeros((8, TQ), F32))

    for d in late_cp:
        d.wait()
    r = r_s[0:1, :].astype(BF16).astype(F32)
    rmax = jnp.max(r, axis=-1, keepdims=True)
    tok = lax.broadcasted_iota(jnp.int32, (1, S), 1)
    idx = jnp.min(jnp.where(r == rmax, tok, S - 1))
    blk = pl.multiple_of((idx // 16) * 16, 16)
    xsel = xn_s[pl.ds(blk, 16), :]
    ffn = dict(y=None, done=False)

    def down(n0, hid):
        for k in range(hid.shape[1] // LANES):
            t = _dot(hid[:, k * LANES:(k + 1) * LANES],
                     wd_s[n0 + k * LANES:n0 + (k + 1) * LANES, :])
            ffn["y"] = t if ffn["y"] is None else ffn["y"] + t
            yield

    def ffn_tasks():
        prev = None
        for n0 in range(0, FT, 4 * LANES):
            n1 = min(n0 + 4 * LANES, FT)
            acc = {}
            for k in range(NG):
                ks = slice(k * LANES, (k + 1) * LANES)
                for name, w in (("g", wg_s), ("u", wu_s)):
                    t = _dot(xsel[:, ks], w[ks, n0:n1])
                    acc[name] = t if k == 0 else acc[name] + t
                    yield
            gate = acc["g"].astype(BF16).astype(F32)
            up = acc["u"].astype(BF16).astype(F32)
            hid = ((gate * jax.nn.sigmoid(gate)).astype(BF16).astype(F32) * up).astype(BF16)
            if prev is not None:
                yield from down(*prev)
            prev = (n0, hid)
        yield
        yield
        yield from down(*prev)
        ffn["done"] = True

    def pv_tasks():
        _, hp, tp, _ = item(NJ - 1, HG - 1)
        st = Step((hp, hp, tp), None, m, sa_s, sb_s)
        for c in range(NC):
            st.do_pv(c)
            if c == NC - 1:
                st.finish()
            yield

    live = [(ffn_tasks(), 3), (pv_tasks(), 1)]

    def fill(drain=False):
        while live:
            gen, rate = live[0]
            if any([next(gen, "end") == "end" for _ in range(rate)]):
                live.pop(0)
            elif not drain:
                return

    sent = 0
    copies = []
    for p in range(S // OP):
        rows = pl.ds(p * OP, OP)
        done = (p + 1) * OP
        if done > S - TQ:
            fill(True)
        a = None
        for k in range(NG):
            if p > 0:
                fill()
            ks = slice(k * LANES, (k + 1) * LANES)
            t = _dot_tn(ot_s[ks, rows], wo_s[ks, :])
            a = t if a is None else a + t
        out_s[rows, :] = (a + res_s[rows, :]).astype(BF16)
        if ffn["done"] and ffn["y"] is not None:
            row = lax.broadcasted_iota(jnp.int32, (16, D), 0) + blk
            upd = jnp.where(row == idx, ffn["y"] * jax.nn.sigmoid(rmax), 0.0)
            b = pl.ds(pl.multiple_of(jnp.minimum(blk, done - 16), 16), 16)
            out_s[b, :] = (out_s[b, :].astype(F32)
                           + jnp.where(blk < done, upd, 0.0)).astype(BF16)
            res_s[pl.ds(blk, 16), :] = res_s[pl.ds(blk, 16), :] + upd
            ffn["y"] = None
        if ffn["done"] and (p + 1 in OUT_DMAS or done == S):
            rr = pl.ds(sent, done - sent)
            copies.append(pltpu.make_async_copy(out_s.at[rr], out_hbm.at[rr],
                                                osems.at[len(copies)]))
            copies[-1].start()
            sent = done
    for d in copies:
        d.wait()


@jax.jit
def pallas_parallel_sum__softmax_full_mha__moe_arch_mod__prompt_kernel(
    A_x: jax.Array,
    A_wqkv: jax.Array,
    A_wo: jax.Array,
    B_x: jax.Array,
    B_w_r: jax.Array,
    B_w_gate: jax.Array,
    B_w_up: jax.Array,
    B_w_down: jax.Array,
):
    del B_x
    B, S, D = A_x.shape
    F = B_w_gate.shape[1]
    assert B == 1
    hbm = pl.BlockSpec(memory_space=pl.ANY)
    out = pl.pallas_call(
        _kernel,
        out_shape=jax.ShapeDtypeStruct((S, D), BF16),
        in_specs=[hbm] * 7,
        out_specs=hbm,
        scratch_shapes=[
            pltpu.VMEM((S, D), BF16), pltpu.VMEM((D, 3 * D), BF16), pltpu.VMEM((D, D), BF16),
            pltpu.VMEM((D,), BF16), pltpu.VMEM((D, F), BF16), pltpu.VMEM((D, F), BF16),
            pltpu.VMEM((F, D), BF16), pltpu.VMEM((S, D), BF16),
            pltpu.VMEM((S, D), BF16), pltpu.VMEM((S, D), F32), pltpu.VMEM((2 * D + 16, D), BF16),
            pltpu.VMEM((D, S), BF16), pltpu.VMEM((D // LANES, S, LANES), BF16),
            pltpu.VMEM((D, S), BF16), pltpu.VMEM((8, S), F32),
            pltpu.VMEM((S, TQ), F32), pltpu.VMEM((S, TQ), F32),
            pltpu.VMEM((D + 16, S), BF16), pltpu.SMEM((1,), jnp.int32),
            pltpu.SemaphoreType.DMA((S // RC + 8,)),
            pltpu.SemaphoreType.DMA((len(OUT_DMAS) + 1,)),
        ],
        compiler_params=pltpu.CompilerParams(vmem_limit_bytes=64 * 1024 * 1024),
        name="fused_block",
    )(A_x.reshape(S, D), A_wqkv, A_wo, B_w_r, B_w_gate, B_w_up, B_w_down)
    return out.reshape(B, S, D)
```
